```python
import os as _os
_os.environ.setdefault("JAX_PLATFORMS", "cpu")
import jax
import jax.numpy as jnp

def _softmax(x, axis=-1):
    return jax.nn.softmax(x, axis=axis)
def _gelu(x):
    return jax.nn.gelu(x, approximate=True)
def _silu(x):
    return jax.nn.silu(x)
def _sigmoid(x):
    return jax.nn.sigmoid(x)
def _layernorm(x, axis=-1, eps=1e-5):
    m = jnp.mean(x, axis=axis, keepdims=True)
    v = jnp.var(x, axis=axis, keepdims=True)
    return (x - m) / jnp.sqrt(v + eps)
def _scatter_add(tgt, idx, src, axis=0):
    return tgt.at[idx].add(src)
def _segment_sum(src, seg, n):
    return jax.ops.segment_sum(src, seg, n)
class _Rng:
    def __init__(self, key):
        self._k = key
    def _next(self):
        self._k, sub = jax.random.split(self._k)
        return sub
    def normal(self, shape):
        return jax.random.normal(self._next(), shape, dtype=jnp.bfloat16)
    def randint(self, lo, hi, shape):
        return jax.random.randint(self._next(), shape, lo, hi, dtype=jnp.int32)
    def uniform(self, shape, lo=0.0, hi=1.0):
        return jax.random.uniform(self._next(), shape, jnp.bfloat16, lo, hi)
    def permutation(self, n):
        return jax.random.permutation(self._next(), n)


kernel_name = 'sequential_preLN__sliding_block__dense_activation_gelu__prompt'

def setup_inputs():
    _rng = _Rng(jax.random.key(int.from_bytes(__import__("os").urandom(4), "little")))
    _w = (lambda a: (lambda t: t.astype(jnp.bfloat16) if jnp.issubdtype(t.dtype, jnp.floating) else t)(jnp.asarray(a)))
    def _A_setup():
        B, S, D = 1, 2048, 640
        return {
            "x": _w((lambda *s: _rng.normal(s) * 0.05)(B, S, D)),
            "wqkv": _w((lambda *s: _rng.normal(s) * 0.05)(D, 3 * D)),
            "wo": _w((lambda *s: _rng.normal(s) * 0.05)(D, D)),
        }
    _A_in = _A_setup()

    def _B_setup():
        B, S, D, F = 1, 2048, 640, 1536
        return {
            "x": _w((lambda *s: _rng.normal(s) * 0.05)(B, S, D)),
            "w1": _w((lambda *s: _rng.normal(s) * 0.8)(D, F) * (D ** -0.5)),
            "b1": _w((lambda *s: _rng.normal(s) * 0.8)(F) * 0.01),
            "w2": _w((lambda *s: _rng.normal(s) * 0.8)(F, D) * (F ** -0.5)),
            "b2": _w((lambda *s: _rng.normal(s) * 0.05)(D) * 0.01),
        }
    _B_in = _B_setup()

    return {
        "A_x": _A_in["x"],
        "A_wqkv": _A_in["wqkv"],
        "A_wo": _A_in["wo"],
        "B_x": _B_in["x"],
        "B_w1": _B_in["w1"],
        "B_b1": _B_in["b1"],
        "B_w2": _B_in["w2"],
        "B_b2": _B_in["b2"],
    }

def reference(A_x, A_wqkv, A_wo, B_x, B_w1, B_b1, B_w2, B_b2):
    def _A_ref(x, wqkv, wo):
        B, S, D = x.shape
        H = 32; Dh = D // H; W = 256
        qkv = (lambda x, *d: x.transpose(*d))((x @ wqkv).reshape(B, S, 3, H, Dh), 2, 0, 3, 1, 4)
        q, k, v = qkv[0], qkv[1], qkv[2]
        scores = jnp.einsum("bhqd,bhkd->bhqk", q, k) * (Dh ** -0.5)
        idx = jnp.arange(S)
        mask = (idx[:, None] - idx[None, :] >= 0) & (idx[:, None] - idx[None, :] < W)
        scores = jnp.where(mask[None, None], scores, -1e9)
        p = _softmax(scores, axis=-1)
        o = jnp.einsum("bhqk,bhkd->bhqd", p, v)
        return (lambda x, *d: x.transpose(*d))(o, 0, 2, 1, 3).reshape(B, S, D) @ wo

    def _B_ref(x, w1, b1, w2, b2):
        h = jnp.einsum("bsd,df->bsf", x, w1) + b1
        h = _gelu(h)
        return jnp.einsum("bsf,fd->bsd", h, w2) + b2

    x = A_x
    h = x + _A_ref(_layernorm(x, axis=-1), A_wqkv, A_wo)
    h2 = h + _B_ref(_layernorm(h, axis=-1), B_w1, B_b1, B_w2, B_b2)
    return h2
```

```python
import functools
import math
import jax
import jax.numpy as jnp
from jax import lax
import jax.experimental.pallas as pl
import jax.experimental.pallas.tpu as pltpu

S, D, F = 2048, 640, 1536
H, DH, W = 32, 20, 256
NG = 8
QB = 128
CH = 32
WIN = W + CH
NSB = S // QB
LOG2E = 1.4426950408889634
NEG = -1e9 * LOG2E
EPS = 1e-5
QSCALE = (DH ** -0.5) * LOG2E
F32 = jnp.float32
BF16 = jnp.bfloat16
U32 = jnp.uint32


def _ln(x):
    m = jnp.mean(x, axis=-1, keepdims=True)
    xc = x - m
    v = jnp.mean(xc * xc, axis=-1, keepdims=True)
    return xc * lax.rsqrt(v + EPS)


def _gelu(x):
    c = math.sqrt(2.0 / math.pi)
    inner = x * (c + (c * 0.044715) * (x * x))
    return (0.5 * x) * (1.0 + jnp.tanh(inner))


def _pk(a):
    return pltpu.bitcast(a.astype(BF16), U32)


def _up(a):
    return pltpu.bitcast(a, BF16)


def _pk2(a, b, rnd):
    ua = lax.bitcast_convert_type(a, U32)
    ub = lax.bitcast_convert_type(b, U32)
    if rnd:
        ua = ua + U32(0x8000)
        ub = ub + U32(0x8000)
    return (ua >> 16) | (ub & U32(0xFFFF0000))


def _pki(a, rnd):
    r, n = a.shape
    a4 = a.reshape(r // 16, 2, 8, n)
    return _pk2(a4[:, 0], a4[:, 1], rnd).reshape(r // 2, n)


def _dot(a, b):
    return jnp.dot(a, b, preferred_element_type=F32)


def _rows(sb):
    if isinstance(sb, int):
        return pl.ds(QB * sb, QB)
    return pl.ds(pl.multiple_of(sb * QB, QB), QB)


def make_kernel(lag=2, plan=None, stage_s=True, stage_d=True):

    def kernel(x_h, wqkv_h, wo_h, w1_h, b1_ref, w2_h, b2_ref, o_h,
               x_s, out_s, wqkv_s, wo_s, w1_s, w2_s, kw_s, vw_s, q_s, ot_s, o_s,
               xsem, wsem, osem, xn_s, xni_s, hn_s, hb_s, gl_s, *s_refs):
        par = {'w': 0, 'rs': 0, 'rd': 0}
        lane1 = lax.broadcasted_iota(jnp.int32, (1, 128), 1)

        def x_copy(sb):
            return pltpu.make_async_copy(x_h.at[0, _rows(sb)], x_s.at[_rows(sb)], xsem.at[sb])

        def o_copy(sb):
            return pltpu.make_async_copy(out_s.at[_rows(sb)], o_h.at[0, _rows(sb)], osem.at[sb])

        def wqkv_copy(i):
            return pltpu.make_async_copy(wqkv_h.at[:, D * i:D * (i + 1)],
                                         wqkv_s.at[:, D * i:D * (i + 1)], wsem.at[i])

        wo_copy = pltpu.make_async_copy(wo_h, wo_s, wsem.at[3])
        w1_copy = pltpu.make_async_copy(w1_h, w1_s, wsem.at[4])
        w2_copy = pltpu.make_async_copy(w2_h, w2_s, wsem.at[5])

        x_copy(0).start()
        wqkv_copy(1).start()
        wqkv_copy(0).start()
        x_copy(1).start()
        wqkv_copy(2).start()
        x_copy(2).start()
        x_copy(3).start()
        wo_copy.start()
        w1_copy.start()
        w2_copy.start()
        for sb in range(4, NSB):
            x_copy(sb).start()

        r32 = lax.broadcasted_iota(jnp.int32, (CH, 128), 0)
        l32 = lax.broadcasted_iota(jnp.int32, (CH, 128), 1) % CH
        tri = r32 > l32
        b0 = (lane1 // CH) % 2 == 0
        b1m = lane1 < 64
        sub8 = lax.broadcasted_iota(jnp.int32, (8, 128), 0) < 4
        zero8 = jnp.zeros((8, 128), U32)
        r16 = lax.broadcasted_iota(jnp.int32, (CH // 2, 128), 0)
        l16 = lax.broadcasted_iota(jnp.int32, (CH // 2, 128), 1) % CH
        rlo = 16 * (r16 // 8) + r16 % 8
        tri_w = (jnp.where(rlo > l16, U32(0x0000FFFF), U32(0))
                 | jnp.where(rlo + 8 > l16, U32(0xFFFF0000), U32(0)))
        ntri_w = ~tri_w
        ones8 = jnp.ones((8, 128), F32)

        def gtile(tiles, g):
            t0, off = divmod(80 * g, 128)
            if off + 80 <= 128:
                return tiles[t0]
            return jnp.where(lane1 >= off, tiles[t0], tiles[t0 + 1])

        def groups_ready(t):
            out = []
            for g in range(NG):
                t0, off = divmod(80 * g, 128)
                tl = t0 if off + 80 <= 128 else t0 + 1
                if tl == t:
                    out.append(g)
            return out

        def qkv_items(sb, nshift):
            st = {'k': {}, 'q': {}, 'vt': {}}

            def ln_item():
                x = x_s[_rows(sb), :].astype(F32)
                xnf = _ln(x)
                xn_s[par['w']] = _pk(xnf)
                xni_s[par['w']] = _pki(xnf, True)

            def k_item(t):
                def f():
                    st['k'][t] = _pk(_dot(_up(xn_s[par['rd']]), wqkv_s[:, D + 128 * t:D + 128 * (t + 1)]))
                    for g in groups_ready(t):
                        if nshift == 2:
                            kw_s[g, 0:64, :] = kw_s[g, 64:128, :]
                        if nshift >= 1:
                            kw_s[g, 64:128, :] = kw_s[g, 128:192, :]
                        kw_s[g, 128:192, :] = gtile(st['k'], g)
                return f

            def v_item(t):
                def f():
                    v = _dot(_up(xni_s[par['rd']]), wqkv_s[:, 2 * D + 128 * t:2 * D + 128 * (t + 1)])
                    st['vt'][t] = v.T
                return f

            def v_store(t):
                def f():
                    for p in range(H // 2):
                        if (40 * p + 39) // 128 == t:
                            rows = []
                            for r8 in range(5):
                                r = 40 * p + 8 * r8
                                rows.append(st['vt'][r // 128][r % 128:r % 128 + 8])
                            full = jnp.concatenate(rows[0:3] + [ones8] + rows[3:5], axis=0)
                            sl = slice(24 * p, 24 * p + 24)
                            if nshift == 2:
                                vw_s[0, sl, :] = vw_s[1, sl, :]
                            if nshift >= 1:
                                vw_s[1, sl, :] = vw_s[2, sl, :]
                            vw_s[2, sl, :] = _pk(full)
                return f

            def q_item(t):
                def f():
                    st['q'][t] = _pk(_dot(_up(xn_s[par['rd']]), wqkv_s[:, 128 * t:128 * (t + 1)]) * QSCALE)
                    for g in groups_ready(t):
                        off = (80 * g) % 128
                        rel = (lane1 - off) % 128
                        qg = gtile(st['q'], g)
                        for j in range(4):
                            hm = (rel >= DH * j) & (rel < DH * (j + 1))
                            pj = jnp.where(hm, qg, U32(0))
                            for c in range(4):
                                s = (j + c) % 4
                                q_s[g, c, 16 * s:16 * (s + 1), :] = pj[16 * c:16 * (c + 1)]
                return f

            return dict(ln=ln_item, k=[k_item(t) for t in range(5)], q=[q_item(t) for t in range(5)],
                        v=[v_item(t) for t in range(5)], vs=[v_store(t) for t in range(5)])

        def conv_item():
            o_s[...] = _pk(ot_s[...].T)

        def post_items(sb, o_val=None, bs=0):
            st = {'h': {}, 'gl': {}}

            def wo_item(t):
                def f():
                    o = _up(o_s[...]) if o_val is None else o_val()
                    a = _dot(o, wo_s[:, 128 * t:128 * (t + 1)])
                    st['h'][t] = x_s[_rows(sb), 128 * t:128 * (t + 1)].astype(F32) + a
                    if t == 4:
                        h = jnp.concatenate([st['h'][i] for i in range(5)], axis=1)
                        hn_s[bs, par['w']] = _pk(_ln(h))
                        hb_s[bs, par['w']] = h + b2_ref[...].astype(F32)
                return f

            def w1_item(t):
                def f():
                    h1 = (_dot(_up(hn_s[bs, par['rd']]), w1_s[:, 128 * t:128 * (t + 1)])
                          + b1_ref[:, 128 * t:128 * (t + 1)].astype(F32))
                    gl_s[bs, par['w'], :, 128 * t:128 * (t + 1)] = _pk(_gelu(h1))
                return f

            def w2_item(t):
                def f():
                    y = _dot(_up(gl_s[bs, par['rd']]), w2_s[:, 128 * t:128 * (t + 1)])
                    y = y + hb_s[bs, par['rd'], :, 128 * t:128 * (t + 1)]
                    out_s[_rows(sb), 128 * t:128 * (t + 1)] = y.astype(BF16)
                return f

            return dict(wo=[wo_item(t) for t in range(5)], w1=[w1_item(t) for t in range(12)],
                        w2=[w2_item(t) for t in range(5)])

        def qk(g, nprev):
            res = []
            for c in range(4):
                qbd = _up(q_s[g, c])
                start = CH * c // 2
                r0 = max(0, W - QB * nprev - CH * c)
                m0 = max(r0, CH)
                parts = [kw_s[g, start + W // 2:start + WIN // 2, :]]
                if r0 == 0:
                    parts.append(kw_s[g, start:start + W // 2, :])
                elif m0 < W:
                    parts.append(kw_s[g, start + m0 // 2:start + W // 2, :])
                kw = jnp.concatenate(parts, axis=0) if len(parts) > 1 else parts[0]
                st = lax.dot_general(_up(kw), qbd, (((1,), (1,)), ((), ())),
                                     preferred_element_type=F32)
                if r0 == 0:
                    merged = jnp.where(tri, st[CH:2 * CH], st[0:CH])
                    mid = st[2 * CH:]
                else:
                    merged = jnp.where(tri, NEG, st[0:CH])
                    mid = st[CH:] if m0 < W else None
                m8 = jnp.max(merged.reshape(4, 8, 128), axis=0)
                if mid is not None:
                    m8 = jnp.maximum(m8, jnp.max(mid.reshape(mid.shape[0] // 8, 8, 128), axis=0))
                m = jnp.max(m8, axis=0, keepdims=True)
                s_s = s_refs[g % 3]
                s_s[par['w'], c, 0:CH, :] = merged
                if mid is not None:
                    s_s[par['w'], c, m0:W, :] = mid
                res.append((m, r0, m0))
            return res

        def pv(g, nprev, res):
            ps = []
            for c in range(4):
                m, r0, m0 = res[c]
                s_s = s_refs[g % 3]
                merged = s_s[par['rs'], c, 0:CH, :]
                mid = s_s[par['rs'], c, m0:W, :] if m0 < W else None
                pm = _pki(jnp.exp2(merged - m), False)
                units = [None] * 18
                plast = pm & ntri_w
                units[16], units[17] = plast[0:8], plast[8:16]
                if r0 == 0:
                    pf = pm & tri_w
                    units[0], units[1] = pf[0:8], pf[8:16]
                if mid is not None:
                    pmid = _pki(jnp.exp2(mid - m), False)
                    for u in range(m0 // 16, 16):
                        k_ = u - m0 // 16
                        units[u] = pmid[8 * k_:8 * (k_ + 1)]
                ps.append(units)
            t_lo = 2 - nprev
            ws = [[] for _ in range(4)]
            for v_ in range(24):
                if v_ // 8 < t_lo:
                    for h in range(4):
                        ws[h].append(None)
                    continue
                X = [ps[c][v_ - 2 * c] if 0 <= v_ - 2 * c < 18 else None for c in range(4)]

                def sel(m_, a, b):
                    if a is None and b is None:
                        return None
                    return jnp.where(m_, zero8 if a is None else a, zero8 if b is None else b)
                T = [sel(b0, X[j], X[(j + 1) % 4]) for j in range(4)]
                for h in range(4):
                    w_ = sel(b1m, T[(-h) % 4], T[(-h + 2) % 4])
                    ws[h].append(zero8 if w_ is None else w_)
            outs = []
            accs = [None] * 4
            for t in range(t_lo, 3):
                for j in range(4):
                    h = 4 * g + j
                    r0_ = 24 * (h // 2) + (0 if h % 2 == 0 else 8)
                    wt = _up(jnp.concatenate(ws[j][8 * t:8 * (t + 1)], axis=0))
                    lhs = _up(vw_s[t, r0_:r0_ + 16, :])
                    d = _dot(lhs, wt)
                    accs[j] = d if accs[j] is None else accs[j] + d
            for j in range(4):
                acc = accs[j]
                if j % 2 == 0:
                    a0, a1, bb, sm = acc[0:8], acc[8:16], acc[16:24], acc[24:32]
                else:
                    bb, sm, a0, a1 = acc[0:8], acc[8:16], acc[16:24], acc[24:32]
                r_ = pl.reciprocal(sm, approx=True)
                inv = r_ * (2.0 - sm * r_)
                tiles = [a0 * inv, a1 * inv, bb * inv]
                if j != 0:
                    tiles = [pltpu.roll(t_, 128 - CH * j, 1) for t_ in tiles]
                outs.append(tiles)
            for pp in range(2):
                e, o = outs[2 * pp], outs[2 * pp + 1]
                t2 = jnp.where(sub8, e[2], o[2])
                blk = jnp.concatenate([e[0], e[1], t2, o[0], o[1]], axis=0)
                r = 80 * g + 40 * pp
                ot_s[r:r + 40, :] = blk

        def stage(sb, nprev, do_qkv, do_post, do_conv):
            head, tail = [], []
            slots = [[] for _ in range(NG)]
            if do_qkv:
                x_copy(sb + 1).wait()
                qi = qkv_items(sb + 1, min(nprev + 1, 2))
            if do_post:
                pi = post_items(sb - 2)
                head += pi['wo']
            if do_conv:
                head.append(conv_item)
            if do_qkv:
                head.append(qi['ln'])
            if do_post:
                for i in range(3):
                    slots[i] += pi['w1'][4 * i:4 * i + 4]
                for i in range(4):
                    slots[3 + i].append(pi['w2'][i])
                tail.append(pi['w2'][4])
            if do_qkv:
                if do_post:
                    kq = {1: [0], 3: [1], 4: [2], 5: [3], 6: [4]}
                    slots[1].append(qi['k'][0])
                    slots[2].append(qi['q'][0])
                    for s_, t in ((3, 1), (4, 2), (5, 3), (6, 4)):
                        slots[s_] += [qi['k'][t], qi['q'][t]]
                    for s_, t in ((3, 0), (4, 1), (5, 2), (6, 3)):
                        slots[s_] += [qi['v'][t], qi['vs'][t]]
                    slots[7].append(qi['v'][4])
                    tail.insert(0, qi['vs'][4])
                else:
                    for s_, t in ((0, 0), (1, 1), (2, 2), (4, 3), (6, 4)):
                        slots[s_] += [qi['k'][t], qi['q'][t]]
                    for s_, t in ((2, 0), (3, 1), (5, 2), (6, 3)):
                        slots[s_] += [qi['v'][t], qi['vs'][t]]
                    slots[7].append(qi['v'][4])
                    tail.insert(0, qi['vs'][4])
            res = {}
            nh = len(head)
            for it in head[:1]:
                it()
            for i in range(lag):
                res[i] = qk(i, nprev)
            for it in head[1:]:
                it()
            for g in range(NG):
                if g + lag < NG:
                    res[g + lag] = qk(g + lag, nprev)
                for it in slots[g]:
                    it()
                pv(g, nprev, res.pop(g))
            for it in tail:
                it()
            if do_post:
                o_copy(sb - 2).start()

        qi = qkv_items(0, 0)
        x_copy(0).wait()
        qi['ln']()
        wqkv_copy(1).wait()
        for it in qi['k']:
            it()
        wqkv_copy(0).wait()
        for it in qi['q']:
            it()
        wqkv_copy(2).wait()
        for t in range(5):
            qi['v'][t]()
            qi['vs'][t]()
        stage(0, 0, True, False, False)
        stage(1, 1, True, False, True)
        wo_copy.wait()
        w1_copy.wait()
        w2_copy.wait()

        def body(sb, carry):
            par['w'] = sb & 1
            par['rs'] = ((sb * 3) & 1) if stage_s else par['w']
            par['rd'] = ((sb * 3) & 1) if stage_d else par['w']
            stage(sb, 2, True, True, True)
            par['w'] = par['rs'] = par['rd'] = 0
            return carry
        lax.fori_loop(2, NSB - 1, body, 0)

        stage(NSB - 1, 2, False, True, True)
        pa = post_items(NSB - 2)
        o_last = {}

        def o_val():
            if 'o' not in o_last:
                o_last['o'] = ot_s[...].T.astype(BF16)
            return o_last['o']
        pb = post_items(NSB - 1, o_val, 1)
        for it in pa['wo'] + pb['wo'] + pa['w1'] + pb['w1'] + pa['w2']:
            it()
        o_copy(NSB - 2).start()
        for it in pb['w2']:
            it()
        o_copy(NSB - 1).start()
        for sb in range(NSB):
            o_copy(sb).wait()

    return kernel


@jax.jit
def pallas_sequential_preLN__sliding_block__dense_activation_gelu__prompt_kernel(
    A_x: jax.Array,
    A_wqkv: jax.Array,
    A_wo: jax.Array,
    B_x: jax.Array,
    B_w1: jax.Array,
    B_b1: jax.Array,
    B_w2: jax.Array,
    B_b2: jax.Array,
):
    anyspec = pl.BlockSpec(memory_space=pl.ANY)
    vspec = pl.BlockSpec(memory_space=pltpu.VMEM)
    return pl.pallas_call(
        make_kernel(stage_s=False, stage_d=False),
        in_specs=[anyspec, anyspec, anyspec, anyspec, vspec, anyspec, vspec],
        out_specs=anyspec,
        out_shape=jax.ShapeDtypeStruct((1, S, D), BF16),
        scratch_shapes=[
            pltpu.VMEM((S, D), BF16), pltpu.VMEM((S, D), BF16),
            pltpu.VMEM((D, 3 * D), BF16), pltpu.VMEM((D, D), BF16),
            pltpu.VMEM((D, F), BF16), pltpu.VMEM((F, D), BF16),
            pltpu.VMEM((NG, 192, 128), U32),
            pltpu.VMEM((3, 384, 128), U32),
            pltpu.VMEM((NG, 4, 64, 128), U32),
            pltpu.VMEM((D, QB), F32),
            pltpu.VMEM((QB // 2, D), U32),
            pltpu.SemaphoreType.DMA((NSB,)),
            pltpu.SemaphoreType.DMA((6,)),
            pltpu.SemaphoreType.DMA((NSB,)),
            pltpu.VMEM((2, QB // 2, D), U32), pltpu.VMEM((2, QB // 2, D), U32),
            pltpu.VMEM((2, 2, QB // 2, D), U32), pltpu.VMEM((2, 2, QB, D), F32),
            pltpu.VMEM((2, 2, QB // 2, F), U32),
        ] + [pltpu.VMEM((2, 4, W, 128), F32) for _ in range(3)],
        compiler_params=pltpu.CompilerParams(vmem_limit_bytes=100 * 1024 * 1024),
    )(A_x, A_wqkv, A_wo, B_w1, B_b1.reshape(1, F), B_w2, B_b2.reshape(1, D))
```

```python
import math
import re

import jax
import jax.numpy as jnp
from jax import lax
import jax.experimental.pallas as pl
import jax.experimental.pallas.tpu as pltpu

S, D, F = 2048, 640, 1536
H, DH, W = 32, 20, 256
NG = 8
QB = 128
CH = 32
WIN = W + CH
NSB = S // QB
NS = 3
LOG2E = 1.4426950408889634
NEG = -1e9 * LOG2E
EPS = 1e-5
QSCALE = (DH ** -0.5) * LOG2E
F32 = jnp.float32
BF16 = jnp.bfloat16
U32 = jnp.uint32

KQ = {t: [g for g in range(NG) if (80 * g + 79) // 128 == t] for t in range(5)}
PAIRS = {t: [p for p in range(H // 2) if (40 * p + 39) // 128 == t] for t in range(5)}


def _ln(x, scale=None):
    m = jnp.mean(x, axis=-1, keepdims=True)
    xc = x - m
    v = jnp.mean(xc * xc, axis=-1, keepdims=True)
    r = lax.rsqrt(v + EPS)
    return xc * (r if scale is None else r * scale)


def _gelu_half(hx):
    c = math.sqrt(2.0 / math.pi)
    inner = hx * (2.0 * c + (8.0 * c * 0.044715) * (hx * hx))
    return hx + hx * jnp.tanh(inner)


def _pk(a):
    return pltpu.bitcast(a.astype(BF16), U32)


def _up(a):
    return pltpu.bitcast(a, BF16)


def _pki(a, rnd=True):
    r, n = a.shape
    a4 = lax.bitcast_convert_type(a.reshape(r // 16, 2, 8, n), U32)
    if rnd:
        a4 = a4 + U32(0x8000)
    return ((a4[:, 0] >> 16) | (a4[:, 1] & U32(0xFFFF0000))).reshape(r // 2, n)


def _dot(a, b):
    return jnp.dot(a, b, preferred_element_type=F32)


def _rows(sb, n=1):
    if isinstance(sb, int):
        return pl.ds(QB * sb, QB * n)
    return pl.ds(pl.multiple_of(sb * QB, QB), QB * n)


def _seq(pre, kinds):
    out = []
    for k in kinds.split():
        if k == 'att':
            for g in range(NG):
                out += ['A%d' % g, 'P%da' % g, 'P%db' % g, 'P%dc' % g]
        elif k == 'v':
            for t in range(5):
                out += ['v%d' % t, 's%d' % t]
        elif k in ('k', 'q', 'w', 'g'):
            out += ['%s%d' % (k, t) for t in range(5)]
        elif k == 'f':
            out += ['f%d' % t for t in range(12)]
        else:
            out.append(k)
    return [pre + n for n in out]


CANON = {
    'q': _seq('a', 'q') + _seq('b', 'q') + ['aA0', 'aA1', 'aA2'],
    'rest': (_seq('a', 'v') + _seq('b', 'v') + _seq('c', 'v q')
             + [n for n in _seq('a', 'att') if n not in ('aA0', 'aA1', 'aA2')] + ['aC']
             + _seq('b', 'att C') + _seq('c', 'att') + _seq('d', 'L k q v')),
    'loop': (_seq('x', 'w C f g att L k q v') + _seq('y', 'w C f g att L k q v')),
    'epi': (_seq('e', 'w C f g O att') + _seq('a', 'w f g O') + _seq('b', 'w f g O')
            + ['cC'] + _seq('c', 'w f') + ['cg0', 'cg1', 'cg2', 'cg3', 'cO', 'cg4', 'cZ']),
}
_UBASE = {'q': {'a': 0}, 'rest': {'a': 0, 'b': 8, 'c': 16}, 'loop': {'x': 0, 'y': 8}, 'epi': {'e': 0}}


def _rw(phase, name):
    h, k, t = re.fullmatch(r'([a-z])([a-zA-Z])(\d*)[abc]?', name).groups()
    t = int(t) if t else None
    R, Wr, C = set(), set(), set()
    pro = phase in ('q', 'rest')
    shift = not (pro and h in 'abc')
    qbuf = {'a': 'qa', 'b': 'qb'}.get(h, 'q') if pro else 'q'
    otbuf = 'ot' + h
    otsrc = 'ot' + h
    if phase == 'loop':
        otsrc = {'x': 'oty', 'y': 'otx'}[h]
    elif phase == 'epi':
        otsrc = {'e': 'oty', 'c': 'ote'}.get(h)
    xn = 'xn%d' % {'b': 1, 'c': 2, 'y': 1}.get(h, 0)
    if k == 'L':
        Wr.add(xn)
    elif k in 'kq':
        R.add(xn)
        Wr.add('%s%s%d' % (h, k, t))
        if t:
            R.add('%s%s%d' % (h, k, t - 1))
        Wr.update((qbuf if k == 'q' else 'kw') + str(g) for g in KQ[t])
    elif k == 'v':
        R.add(xn)
        Wr.add('%sv%d' % (h, t))
    elif k == 's':
        R.add('%sv%d' % (h, t))
        if t:
            R.add('%sv%d' % (h, t - 1))
        tiles = range(3) if shift else ['abc'.index(h)]
        Wr.update('vw%d_%d' % (p, i) for p in PAIRS[t] for i in tiles)
    elif k == 'w':
        R.add('ob' if (phase, h) == ('epi', 'b') else 'oa')
        Wr.add('%sh%d' % (h, t))
        if t == 4:
            R.update('%sh%d' % (h, i) for i in range(4))
            Wr.add(h + 'hn')
    elif k == 'C':
        R.update(otsrc + str(g) for g in range(NG))
        if phase == 'rest':
            Wr.add({'a': 'oa', 'b': 'ob'}[h])
        elif (phase, h) == ('epi', 'c'):
            Wr.add('oa')
        else:
            Wr.update(('oa', 'ob'))
    elif k == 'f':
        R.add(h + 'hn')
        Wr.add('%sgl%d' % (h, t))
    elif k == 'g':
        R.add(h + 'hn')
        R.update('%sgl%d' % (h, i) for i in range(12))
        Wr.add('%sout%d' % (h, t))
    elif k in 'OZ':
        R.update('%sout%d' % (h, i) for i in range(5) if not (h == 'c' and (i == 4) != (k == 'Z')))
    elif k == 'A':
        R.update(('kw%d' % t, qbuf + str(t)))
        Wr.update(('S%d' % ((_UBASE[phase][h] + t) % NS), '%sm%d' % (h, t)))
    elif k == 'P':
        ntile = 'abc'.index(h) + 1 if pro else 3
        R.update(('S%d' % ((_UBASE[phase][h] + t) % NS), '%sm%d' % (h, t)))
        R.update('vw%d_%d' % (p, i) for p in (2 * t, 2 * t + 1) for i in range(ntile))
        C.add((h, otbuf + str(t)))
    else:
        raise ValueError(name)
    return R, Wr, C


def _conflicts(phase):
    base = CANON[phase]
    info = {n: _rw(phase, n) for n in base}
    out = []
    for i, a in enumerate(base):
        Ra, Wa, Ca = info[a]
        ca = {x for _, x in Ca}
        for b in base[i + 1:]:
            Rb, Wb, Cb = info[b]
            cb = {x for _, x in Cb}
            if (Wa & (Rb | Wb | cb) or Wb & (Ra | ca) or ca & Rb or cb & Ra
                    or (ca & cb and Ca != Cb)):
                out.append((a, b))
    return out


def plan_ok(phase, plan):
    pos = {n: i for i, n in enumerate(plan)}
    if sorted(plan) != sorted(CANON[phase]):
        return False
    return all(pos[a] < pos[b] for a, b in _conflicts(phase))


PLANS = {
    'q': (
        "aq0 bq0 aq1 aq2 aq3 bq1 bq2 bq3 aA1 aq4 aA2 bq4 aA0 "
    ),
    'rest': (
        "av0 av1 as0 aP0a av4 as1 aP1b aP0b av2 av3 aP0c aA3 bv1 as3 bv0 aP1a as4 bs1 aP1c aA4 "
        "as2 aP2b aP2a aP3c aP2c aA5 aP3a aP3b bv2 aA6 aP4a bs2 aP6a bv3 bs0 aP4b bs3 bv4 aP4c "
        "aA7 aP5b bs4 aP5c aP5a aP6c bA0 aP6b bP0b bA1 aP7c aP7a aP7b bA2 cv0 bP0a bP0c aC bA3 "
        "cs0 cv1 bP1a bP1c cs1 bP1b bP3a bA4 bP2a cv2 bP2c bP2b bA5 cv3 cs3 bP3c cs2 bP3b bA6 "
        "bP4b cq0 cv4 bP4a cs4 bP4c bA7 cq1 bP5a bP5b bP5c bP6b cq2 bP7a cq3 bP7c bP6c cq4 bP7b "
        "cA0 dL bP6a cA1 dq0 bC cA2 cP0a dk0 cP1c cP0b dk1 dq1 cP0c cP1a cP1b cA3 dk2 cP2b dq2 "
        "cP2c dv1 cP3c dv0 cP2a cA4 ds1 cP3a ds0 cA5 cP3b dq3 cP4c cP4a dk3 cP4b dv3 cA6 dv2 cP5a "
        "cP5b cP5c ds2 cA7 cP6c dv4 cP6a cP6b dk4 ds3 cP7c cP7a cP7b ds4 dq4 "
    ),
    'loop': (
        "xw2 xL xw3 xw1 xw0 xw4 xA1 xA0 xC xP0c xk0 xf0 xq0 xP0a xP0b xA2 xP1b xP2c xk1 xf1 xq1 "
        "xP1c xP1a xf3 xf4 xf5 xf6 xA3 xf2 xP2a xP3c xq2 xP2b xv0 xk2 xf7 xA4 xf8 xP3a xv1 xP4c "
        "xP3b xA5 xf11 xf10 xf9 xs0 xP4a xq3 xP4b xA6 xs1 xv2 xP5c xk3 xP6c xg0 xs2 xP5a xA7 xP7c "
        "xg1 xP6a xk4 xP6b xg2 xg3 xv3 xv4 xq4 xP7b xP7a xP5b yw0 xs4 xs3 yL yw3 yw2 yw1 yw4 yA0 "
        "yA1 xg4 yk0 yC yP0c yf0 yq0 yA2 yP0a yP0b yk1 yq1 yP1c yP2c yf1 yP1a yP1b yf5 yf2 yf4 "
        "yA3 yf3 yq2 yk2 yP2a yf6 yP2b yA4 yf7 yP3c yv0 yA5 yP3a yf8 yv1 yP3b yf9 yf10 yf11 yP4c "
        "ys0 yg0 yP4a yq3 yP4b ys1 yA6 yv2 yP5c yk3 yP5a yA7 yk4 yg1 yP6c yP5b yP6a yg3 yP6b yP7c "
        "yg2 yv3 yv4 yq4 ys3 ys2 yP7b yP7a ys4 yg4 "
    ),
    'epi': (
        "ew0 ew1 ew2 ew3 ew4 eA1 eA0 eA2 eC eP0c eP0a eP0b eA3 eP1c eP1a ef0 eP1b eA4 ef5 eP2a "
        "ef1 eP2c ef3 ef2 ef4 ef7 eP2b eA5 eP4a ef6 ef8 ef9 eP3c eP3a eP3b ef10 eA6 ef11 eP4c eg0 "
        "eP4b eP5c eA7 eP5a eP5b eP7a eg1 eP6a eP6c eP6b eg3 eP7c aw3 eg2 eP7b aw2 eg4 eO aw0 aw1 "
        "aw4 bw3 cC bw0 bw2 bw1 af2 af8 af4 bw4 af5 cw0 af6 af1 af3 af9 af10 af11 cw1 cw3 cw2 af0 "
        "bf0 af7 cw4 bf2 ag2 bf1 bf5 bf10 ag0 bf7 bf8 bf9 cf3 cf2 cf4 ag1 ag4 bf6 bf3 bf4 cf1 "
        "bf11 ag3 aO cf0 cf5 cf7 cf8 bg0 cf10 cf9 cf11 cf6 bg1 bg2 bg4 bg3 cg0 cg3 bO cg1 cg2 cO "
        "cg4 cZ "
    ),
}


def make_kernel():
    plans = PLANS
    for ph, p in plans.items():
        assert plan_ok(ph, p.split()), ph

    def kernel(x_h, wqkv_h, wo_h, w1_h, b1_h, w2_h, b2_h, o_h,
               x_s, out_s, wqkv_s, wo_s, w1_s, w2_s, b1_s, b2_s, b1f_s, b2f_s,
               kw_s, vw_s, q_s, ot_s, oa_s, ob_s, isem, osem,
               xn_s, xni_s, hn_s, hb_s, gl_s, *s_refs):
        par = {'p': 0}
        lane1 = lax.broadcasted_iota(jnp.int32, (1, 128), 1)

        def x_copy(sb, n=1):
            return pltpu.make_async_copy(x_h.at[0, _rows(sb, n)], x_s.at[_rows(sb, n)],
                                         isem.at[16 + sb])

        def o_copy(sb, lo=0, hi=D, sem=None, n=1):
            return pltpu.make_async_copy(out_s.at[_rows(sb, n), lo:hi],
                                         o_h.at[0, _rows(sb, n), lo:hi],
                                         osem.at[sb if sem is None else sem])

        def w_copy(i):
            lo, hi = ((D, D + 256), (D + 256, 2 * D), (0, D), (2 * D, 3 * D))[i]
            return pltpu.make_async_copy(wqkv_h.at[:, lo:hi], wqkv_s.at[:, lo:hi], isem.at[i])

        def late_copies():
            return [pltpu.make_async_copy(wo_h, wo_s, isem.at[4]),
                    pltpu.make_async_copy(b1_h, b1_s, isem.at[5]),
                    pltpu.make_async_copy(b2_h, b2_s, isem.at[6]),
                    pltpu.make_async_copy(w1_h, w1_s, isem.at[7]),
                    pltpu.make_async_copy(w2_h, w2_s, isem.at[8])]

        for sb in range(3):
            x_copy(sb).start()
        for i in range(3):
            w_copy(i).start()

        r32 = lax.broadcasted_iota(jnp.int32, (CH, 128), 0)
        l32 = lax.broadcasted_iota(jnp.int32, (CH, 128), 1) % CH
        tri = r32 > l32
        b0 = (lane1 // CH) % 2 == 0
        b1m = lane1 < 64
        sub8 = lax.broadcasted_iota(jnp.int32, (8, 128), 0) < 4
        zero8 = jnp.zeros((8, 128), U32)
        r16 = lax.broadcasted_iota(jnp.int32, (CH // 2, 128), 0)
        l16 = lax.broadcasted_iota(jnp.int32, (CH // 2, 128), 1) % CH
        rlo = 16 * (r16 // 8) + r16 % 8
        tri_w = (jnp.where(rlo > l16, U32(0x0000FFFF), U32(0))
                 | jnp.where(rlo + 8 > l16, U32(0xFFFF0000), U32(0)))
        ntri_w = ~tri_w
        ones8 = jnp.ones((8, 128), F32)

        def gtile(tiles, g):
            t0, off = divmod(80 * g, 128)
            if off + 80 <= 128:
                return tiles[t0]
            return jnp.where(lane1 >= off, tiles[t0], tiles[t0 + 1])

        def qkv_items(sb, tile=None, bs=0, qs=0):
            st = {'k': {}, 'q': {}, 'vt': {}}
            it = {}

            def ln_item():
                xnf = _ln(x_s[_rows(sb), :].astype(F32))
                xn_s[bs, par['p']] = _pk(xnf)
                xni_s[bs, par['p']] = _pki(xnf)
            it['L'] = ln_item

            def k_item(t):
                st['k'][t] = _pk(_dot(_up(xn_s[bs, par['p']]),
                                      wqkv_s[:, D + 128 * t:D + 128 * (t + 1)]))
                for g in KQ[t]:
                    if tile is None:
                        kw_s[g, 0:128, :] = kw_s[g, 64:192, :]
                        kw_s[g, 128:192, :] = gtile(st['k'], g)
                    else:
                        kw_s[g, 64 * tile:64 * (tile + 1), :] = gtile(st['k'], g)

            def q_item(t):
                st['q'][t] = _pk(_dot(_up(xn_s[bs, par['p']]),
                                      wqkv_s[:, 128 * t:128 * (t + 1)]) * QSCALE)
                for g in KQ[t]:
                    rel = (lane1 - (80 * g) % 128) % 128
                    qg = gtile(st['q'], g)
                    for j in range(4):
                        pj = jnp.where((rel >= DH * j) & (rel < DH * (j + 1)), qg, U32(0))
                        for c in range(4):
                            s = (j + c) % 4
                            q_s[qs, g, c, 16 * s:16 * (s + 1), :] = pj[16 * c:16 * (c + 1)]

            def v_item(t):
                v = _dot(_up(xni_s[bs, par['p']]), wqkv_s[:, 2 * D + 128 * t:2 * D + 128 * (t + 1)])
                st['vt'][t] = v.T

            def v_store(t):
                for p in PAIRS[t]:
                    rows = []
                    for r8 in range(5):
                        r = 40 * p + 8 * r8
                        rows.append(st['vt'][r // 128][r % 128:r % 128 + 8])
                    full = jnp.concatenate(rows[0:3] + [ones8] + rows[3:5], axis=0)
                    sl = slice(24 * p, 24 * p + 24)
                    if tile is None:
                        vw_s[0, sl, :] = vw_s[1, sl, :]
                        vw_s[1, sl, :] = vw_s[2, sl, :]
                        vw_s[2, sl, :] = _pk(full)
                    else:
                        vw_s[tile, sl, :] = _pk(full)

            for t in range(5):
                it['k%d' % t] = lambda t=t: k_item(t)
                it['q%d' % t] = lambda t=t: q_item(t)
                it['v%d' % t] = lambda t=t: v_item(t)
                it['s%d' % t] = lambda t=t: v_store(t)
            return it

        def conv(dst, ots):
            dst[...] = _pk(ot_s[ots].T)

        def conv_fifo(ots):
            oa_s[...] = ob_s[...]
            conv(ob_s, ots)

        def post_items(sb, o_src, bs=0):
            st = {}
            it = {}

            def wo_item(t):
                a = _dot(_up(o_src[...]), wo_s[:, 128 * t:128 * (t + 1)])
                st[t] = x_s[_rows(sb), 128 * t:128 * (t + 1)].astype(F32) + a
                if t == 4:
                    h = jnp.concatenate([st[i] for i in range(5)], axis=1)
                    hn_s[bs, par['p']] = _pk(_ln(h, 0.5))
                    hb_s[bs, par['p']] = h + b2f_s[...]

            def w1_item(t):
                hx = (_dot(_up(hn_s[bs, par['p']]), w1_s[:, 128 * t:128 * (t + 1)])
                      + b1f_s[:, 128 * t:128 * (t + 1)])
                gl_s[bs, par['p'], :, 128 * t:128 * (t + 1)] = _pk(_gelu_half(hx))

            def w2_item(t):
                y = _dot(_up(gl_s[bs, par['p']]), w2_s[:, 128 * t:128 * (t + 1)])
                y = y + hb_s[bs, par['p'], :, 128 * t:128 * (t + 1)]
                out_s[_rows(sb), 128 * t:128 * (t + 1)] = y.astype(BF16)

            for t in range(5):
                it['w%d' % t] = lambda t=t: wo_item(t)
                it['g%d' % t] = lambda t=t: w2_item(t)
            for t in range(12):
                it['f%d' % t] = lambda t=t: w1_item(t)
            return it

        def att_items(nprev=2, qs=0, ots=0, ubase=0):
            res, wres, accd, done, it = {}, {}, {}, {}, {}
            toff = 2 - nprev

            def qk(g):
                out = []
                s_s = s_refs[(ubase + g) % NS]
                for c in range(4):
                    qbd = _up(q_s[qs, g, c])
                    start = CH * c // 2 - 64 * toff
                    r0 = max(0, W - QB * nprev - CH * c)
                    m0 = max(r0, CH)
                    parts = [kw_s[g, start + W // 2:start + WIN // 2, :]]
                    if r0 == 0:
                        parts.append(kw_s[g, start:start + W // 2, :])
                    elif m0 < W:
                        parts.append(kw_s[g, start + m0 // 2:start + W // 2, :])
                    kw = jnp.concatenate(parts, axis=0) if len(parts) > 1 else parts[0]
                    st = lax.dot_general(_up(kw), qbd, (((1,), (1,)), ((), ())),
                                         preferred_element_type=F32)
                    if r0 == 0:
                        merged = jnp.where(tri, st[CH:2 * CH], st[0:CH])
                        mid = st[2 * CH:]
                    else:
                        merged = jnp.where(tri, NEG, st[0:CH])
                        mid = st[CH:] if m0 < W else None
                    m8 = jnp.max(merged.reshape(4, 8, 128), axis=0)
                    s_s[par['p'], c, 0:CH, :] = merged
                    if mid is not None:
                        m8 = jnp.maximum(m8, jnp.max(mid.reshape(mid.shape[0] // 8, 8, 128), axis=0))
                        s_s[par['p'], c, m0:W, :] = mid
                    out.append((jnp.max(m8, axis=0, keepdims=True), r0, m0))
                res[g] = out

            def softmax(g):
                s_s = s_refs[(ubase + g) % NS]
                ps = []
                for c in range(4):
                    m, r0, m0 = res[g][c]
                    pm = _pki(jnp.exp2(s_s[par['p'], c, 0:CH, :] - m), False)
                    units = [None] * 18
                    plast = pm & ntri_w
                    units[16], units[17] = plast[0:8], plast[8:16]
                    if r0 == 0:
                        pf = pm & tri_w
                        units[0], units[1] = pf[0:8], pf[8:16]
                    if m0 < W:
                        pmid = _pki(jnp.exp2(s_s[par['p'], c, m0:W, :] - m), False)
                        for u in range(m0 // 16, 16):
                            k_ = u - m0 // 16
                            units[u] = pmid[8 * k_:8 * (k_ + 1)]
                    ps.append(units)

                def sel(m_, a, b):
                    if a is None and b is None:
                        return None
                    return jnp.where(m_, zero8 if a is None else a, zero8 if b is None else b)

                ws = [[None] * 24 for _ in range(4)]
                for v_ in range(8 * toff, 24):
                    X = [ps[c][v_ - 2 * c] if 0 <= v_ - 2 * c < 18 else None for c in range(4)]
                    T = [sel(b0, X[j], X[(j + 1) % 4]) for j in range(4)]
                    for h in range(4):
                        w_ = sel(b1m, T[(-h) % 4], T[(-h + 2) % 4])
                        ws[h][v_] = zero8 if w_ is None else w_
                wres[g] = ws

            def pv(g, t):
                if g not in wres:
                    softmax(g)
                accs = accd.setdefault(g, [None] * 4)
                if t >= toff:
                    for j in range(4):
                        h = 4 * g + j
                        r0_ = 24 * (h // 2) + (0 if h % 2 == 0 else 8)
                        wt = _up(jnp.concatenate(wres[g][j][8 * t:8 * (t + 1)], axis=0))
                        d = _dot(_up(vw_s[t - toff, r0_:r0_ + 16, :]), wt)
                        accs[j] = d if accs[j] is None else accs[j] + d
                done[g] = done.get(g, 0) + 1
                if done[g] == 3:
                    finish(g)

            def finish(g):
                outs = []
                for j in range(4):
                    acc = accd[g][j]
                    if j % 2 == 0:
                        a0, a1, bb, sm = acc[0:8], acc[8:16], acc[16:24], acc[24:32]
                    else:
                        bb, sm, a0, a1 = acc[0:8], acc[8:16], acc[16:24], acc[24:32]
                    r_ = pl.reciprocal(sm, approx=True)
                    inv = r_ * (2.0 - sm * r_)
                    tiles = [a0 * inv, a1 * inv, bb * inv]
                    if j != 0:
                        tiles = [pltpu.roll(t_, 128 - CH * j, 1) for t_ in tiles]
                    outs.append(tiles)
                for pp in range(2):
                    e, o = outs[2 * pp], outs[2 * pp + 1]
                    t2 = jnp.where(sub8, e[2], o[2])
                    r = 80 * g + 40 * pp
                    ot_s[ots, r:r + 40, :] = jnp.concatenate([e[0], e[1], t2, o[0], o[1]], axis=0)

            for g in range(NG):
                it['A%d' % g] = lambda g=g: qk(g)
                for t in range(3):
                    it['P%d%s' % (g, 'abc'[t])] = lambda g=g, t=t: pv(g, t)
            return it

        def run(names, items):
            for n in names.split():
                items[n]()

        def streams(**kw):
            out = {}
            for p, ds in kw.items():
                for d in ds:
                    out.update({p + k: v for k, v in d.items()})
            return out

        pro = streams(
            a=[qkv_items(0, tile=0, bs=0, qs=1), att_items(0, qs=1, ots=1, ubase=0),
               {'C': lambda: conv(oa_s, 1)}],
            b=[qkv_items(1, tile=1, bs=1, qs=2), att_items(1, qs=2, ots=2, ubase=8),
               {'C': lambda: conv(ob_s, 2)}],
            c=[qkv_items(2, tile=2, bs=2, qs=0), att_items(2, ots=3, ubase=16)],
            d=[qkv_items(3, bs=0)])
        for sb in range(3):
            x_copy(sb).wait()
        w_copy(3).start()
        x_copy(3).start()
        for c in late_copies():
            c.start()
        run("aL bL cL", pro)
        w_copy(0).wait()
        for sb in range(4, NSB, 2):
            x_copy(sb, 2).start()
        run("ak0 ak1 bk0 bk1 ck0 ck1", pro)
        w_copy(1).wait()
        run("ak2 ak3 ak4 bk2 bk3 bk4 ck2 ck3 ck4", pro)
        w_copy(2).wait()
        run(plans['q'], pro)
        w_copy(3).wait()
        x_copy(3).wait()
        run(plans['rest'], pro)
        for c in late_copies():
            c.wait()
        b1f_s[...] = b1_s[...].astype(F32).reshape(1, F) * 0.5
        b2f_s[...] = b2_s[...].astype(F32).reshape(1, D)

        def body(i, carry):
            sb0 = 3 + 2 * i
            par['p'] = i & 1
            x_copy(sb0 + 1, 2).wait()
            items = streams(**{
                'xy'[u]: [att_items(ots=3 * u, ubase=8 * u), qkv_items(sb0 + u + 1, bs=u),
                          post_items(sb0 + u - 3, oa_s, bs=u),
                          {'C': lambda u=u: conv_fifo(3 - 3 * u)}]
                for u in range(2)})
            run(plans['loop'], items)
            o_copy(sb0 - 3, n=2).start()
            par['p'] = 0
            return carry
        lax.fori_loop(0, (NSB - 4) // 2, body, 0)

        last = NSB - 1
        epi = streams(
            e=[att_items(), post_items(last - 3, oa_s, 0),
               {'C': lambda: conv_fifo(3), 'O': lambda: o_copy(last - 3).start()}],
            a=[post_items(last - 2, oa_s, 1), {'O': lambda: o_copy(last - 2).start()}],
            b=[post_items(last - 1, ob_s, 2), {'O': lambda: o_copy(last - 1).start()}],
            c=[post_items(last, oa_s, 3),
               {'C': lambda: conv(oa_s, 0), 'O': lambda: o_copy(last, 0, 512).start(),
                'Z': lambda: o_copy(last, 512, D, NSB).start()}])
        run(plans['epi'], epi)
        for sb in range(0, last - 3, 2):
            o_copy(sb, n=2).wait()
        for sb in range(last - 3, last):
            o_copy(sb).wait()
        o_copy(last, 0, 512).wait()
        o_copy(last, 512, D, NSB).wait()

    return kernel


@jax.jit
def pallas_sequential_preLN__sliding_block__dense_activation_gelu__prompt_kernel(
    A_x: jax.Array,
    A_wqkv: jax.Array,
    A_wo: jax.Array,
    B_x: jax.Array,
    B_w1: jax.Array,
    B_b1: jax.Array,
    B_w2: jax.Array,
    B_b2: jax.Array,
):
    del B_x
    assert A_x.shape == (1, S, D) and A_wqkv.shape == (D, 3 * D) and A_wo.shape == (D, D)
    assert B_w1.shape == (D, F) and B_w2.shape == (F, D)
    assert B_b1.shape == (F,) and B_b2.shape == (D,)
    anyspec = pl.BlockSpec(memory_space=pl.ANY)
    return pl.pallas_call(
        make_kernel(),
        in_specs=[anyspec] * 7,
        out_specs=anyspec,
        out_shape=jax.ShapeDtypeStruct((1, S, D), BF16),
        scratch_shapes=[
            pltpu.VMEM((S, D), BF16), pltpu.VMEM((S, D), BF16),
            pltpu.VMEM((D, 3 * D), BF16), pltpu.VMEM((D, D), BF16),
            pltpu.VMEM((D, F), BF16), pltpu.VMEM((F, D), BF16),
            pltpu.VMEM((F,), BF16), pltpu.VMEM((D,), BF16),
            pltpu.VMEM((1, F), F32), pltpu.VMEM((1, D), F32),
            pltpu.VMEM((NG, 192, 128), U32),
            pltpu.VMEM((3, 384, 128), U32),
            pltpu.VMEM((3, NG, 4, 64, 128), U32),
            pltpu.VMEM((4, D, QB), F32),
            pltpu.VMEM((QB // 2, D), U32), pltpu.VMEM((QB // 2, D), U32),
            pltpu.SemaphoreType.DMA((16 + NSB,)),
            pltpu.SemaphoreType.DMA((NSB + 1,)),
            pltpu.VMEM((3, 2, QB // 2, D), U32), pltpu.VMEM((3, 2, QB // 2, D), U32),
            pltpu.VMEM((4, 2, QB // 2, D), U32), pltpu.VMEM((4, 2, QB, D), F32),
            pltpu.VMEM((4, 2, QB // 2, F), U32),
        ] + [pltpu.VMEM((2, 4, W, 128), F32) for _ in range(NS)],
        compiler_params=pltpu.CompilerParams(vmem_limit_bytes=100 * 1024 * 1024),
    )(A_x, A_wqkv, A_wo, B_w1, B_b1, B_w2, B_b2)
```
